```python
import os as _os
_os.environ.setdefault('JAX_PLATFORMS', 'cpu')
import jax
import jax.numpy as jnp

def _softmax(x, axis=-1):
    return jax.nn.softmax(x, axis=axis)

def _gelu(x):
    return jax.nn.gelu(x, approximate=True)

def _silu(x):
    return jax.nn.silu(x)

def _sigmoid(x):
    return jax.nn.sigmoid(x)

def _layernorm(x, axis=-1, eps=1e-05):
    m = jnp.mean(x, axis=axis, keepdims=True)
    v = jnp.var(x, axis=axis, keepdims=True)
    return (x - m) / jnp.sqrt(v + eps)

def _scatter_add(tgt, idx, src, axis=0):
    return tgt.at[idx].add(src)

def _segment_sum(src, seg, n):
    return jax.ops.segment_sum(src, seg, n)

class _Rng:

    def __init__(self, key):
        self._k = key

    def _next(self):
        self._k, sub = jax.random.split(self._k)
        return sub

    def normal(self, shape):
        return jax.random.normal(self._next(), shape, dtype=jnp.bfloat16)

    def randint(self, lo, hi, shape):
        return jax.random.randint(self._next(), shape, lo, hi, dtype=jnp.int32)

    def uniform(self, shape, lo=0.0, hi=1.0):
        return jax.random.uniform(self._next(), shape, jnp.bfloat16, lo, hi)

    def permutation(self, n):
        return jax.random.permutation(self._next(), n)
kernel_name = 'adaLN_cond__memory_aug_recurrent_mem_tr__moe_arch_mod__prompt'

def setup_inputs():
    _rng = _Rng(jax.random.key(int.from_bytes(__import__("os").urandom(4), "little")))
    _w = lambda a: (lambda t: t.astype(jnp.bfloat16) if jnp.issubdtype(t.dtype, jnp.floating) else t)(jnp.asarray(a))

    def _A_setup():
        B, S, Dm = (1, 2048, 448)
        H, Dh = (16, 256)
        M, seg = (8, 32)
        seg = min(seg, S)
        S = S // seg * seg
        return {'x': _w((lambda *s: _rng.normal(s) * 0.05)(B, S, Dm)), 'mem0': _w((lambda *s: _rng.normal(s) * 0.4)(B, M, Dm)), 'Wq': _w((lambda *s: _rng.normal(s) * 1.6)(Dm, H, Dh) * Dm ** (-0.5)), 'Wk': _w((lambda *s: _rng.normal(s) * 1.6)(Dm, H, Dh) * Dm ** (-0.5)), 'Wv': _w((lambda *s: _rng.normal(s) * 0.4)(Dm, H, Dh) * Dm ** (-0.5)), 'Wo': _w((lambda *s: _rng.normal(s) * 0.4)(H, Dh, Dm) * (H * Dh) ** (-0.5)), 'seg_len': seg}
    _A_in = _A_setup()

    def _B_setup():
        B, S, D, F, C = (1, 2048, 448, 1792, 1)
        return {'x': _w((lambda *s: _rng.normal(s) * 0.05)(B, S, D)), 'w_r': _w((lambda *s: _rng.normal(s) * 0.05)(D)), 'w_gate': _w((lambda *s: _rng.normal(s) * 0.05)(D, F)), 'w_up': _w((lambda *s: _rng.normal(s) * 0.05)(D, F)), 'w_down': _w((lambda *s: _rng.normal(s) * 0.05)(F, D))}
    _B_in = _B_setup()
    return {'A_x': _A_in['x'], 'A_mem0': _A_in['mem0'], 'A_Wq': _A_in['Wq'], 'A_Wk': _A_in['Wk'], 'A_Wv': _A_in['Wv'], 'A_Wo': _A_in['Wo'], 'A_seg_len': _A_in['seg_len'], 'B_x': _B_in['x'], 'B_w_r': _B_in['w_r'], 'B_w_gate': _B_in['w_gate'], 'B_w_up': _B_in['w_up'], 'B_w_down': _B_in['w_down'], 'c': _w((lambda *s: _rng.normal(s) * 0.05)(1, 448) * 8.0), 'w_mod': _w((lambda *s: _rng.normal(s) * 0.05)(448, 6 * 448) * 448 ** (-0.5) * 8.0)}

def reference(A_x, A_mem0, A_Wq, A_Wk, A_Wv, A_Wo, A_seg_len, B_x, B_w_r, B_w_gate, B_w_up, B_w_down, c, w_mod):

    def _A_ref(x, mem0, Wq, Wk, Wv, Wo, seg_len):
        B, S, Dm = x.shape
        H, Dh = (Wq.shape[1], Wq.shape[2])
        M = mem0.shape[1]
        scale = Dh ** (-0.5)
        n_seg = S // seg_len
        L = M + seg_len
        idx = jnp.arange(L)
        mask = (idx[:, None] < M) | (idx[:, None] >= idx[None, :])
        mem = mem0
        outs = []
        for s in range(n_seg):
            xs = x[:, s * seg_len:(s + 1) * seg_len, :].copy()
            h = jnp.concatenate([mem, xs], axis=1)
            q = jnp.einsum('btd,dhe->bhte', h, Wq)
            k = jnp.einsum('btd,dhe->bhte', h, Wk)
            v = jnp.einsum('btd,dhe->bhte', h, Wv)
            scores = jnp.einsum('bhqe,bhke->bhqk', q, k) * scale
            scores = jnp.where(mask[None, None], scores, -1000000000.0)
            p = _softmax(scores, axis=-1)
            o = jnp.einsum('bhqk,bhke->bhqe', p, v)
            o = jnp.einsum('bhte,hed->btd', o, Wo)
            mem = o[:, :M, :].copy()
            outs.append(o[:, M:, :])
        return jnp.concatenate(outs, axis=1)

    def _B_ref(x, w_r, w_gate, w_up, w_down):
        B, S, D = x.shape
        C = 1
        r = x @ w_r
        idx = jnp.argsort(-r, axis=-1)[:, :C]
        idx_e = jnp.repeat(idx.reshape(B, C, 1), D, axis=2)
        x_sel = jnp.take_along_axis(x, idx_e, axis=1)
        g = _silu(x_sel @ w_gate)
        u = x_sel @ w_up
        y = g * u @ w_down
        r_sel = _sigmoid(jnp.take_along_axis(r, idx, axis=1))
        y = y * r_sel.reshape(B, C, 1)
        b_off = (jnp.arange(B) * S).reshape(B, 1)
        flat_idx = (idx + b_off).reshape(B * C)
        zero = (x * 0.0).reshape(B * S, D)
        upd = _scatter_add(zero, flat_idx, y.reshape(B * C, D), axis=0)
        return x + upd.reshape(B, S, D)
    x = A_x
    mod = (_silu(c) @ w_mod).reshape(c.shape[0], 6, 1, -1)
    sa, ca, ga, sb, cb, gb = (mod[:, 0].copy(), mod[:, 1].copy(), mod[:, 2].copy(), mod[:, 3].copy(), mod[:, 4].copy(), mod[:, 5].copy())
    h = _layernorm(x, axis=-1) * (1 + ca) + sa
    x = x + ga * _A_ref(h, A_mem0, A_Wq, A_Wk, A_Wv, A_Wo, A_seg_len)
    h = _layernorm(x, axis=-1) * (1 + cb) + sb
    x = x + gb * _B_ref(h, B_w_r, B_w_gate, B_w_up, B_w_down)
    return x
```

```python
import functools

import jax
import jax.numpy as jnp
from jax import lax
import jax.experimental.pallas as pl
import jax.experimental.pallas.tpu as pltpu

F32 = jnp.float32
BF16 = jnp.bfloat16
U32 = jnp.uint32

D = 448
DP = 512
H = 16
E = 256
M = 8
SEG = 32
S = 2048
F = 1792
G = 128
NG = S // G
NT_DIMS = (((1,), (1,)), ((), ()))
HALF = H * D // 128
NEG = -1000000000.0


def _dot(a, b):
    return jnp.dot(a, b, preferred_element_type=F32)


def _dot_nt(a, b):
    return lax.dot_general(a, b, NT_DIMS, preferred_element_type=F32)


def _round_bf16(x):
    return x.astype(BF16).astype(F32)


def _pack(x):
    return pltpu.bitcast(x.astype(BF16), U32)


def _unpack(x):
    return pltpu.bitcast(x, BF16)


def _dup_rows(w):
    return jnp.concatenate([w, w[384:448]], axis=0)


def _group8(x, op, lane):
    for s in (1, 2, 4):
        partner = jnp.where((lane & s) == 0, pltpu.roll(x, 128 - s, 1), pltpu.roll(x, s, 1))
        x = op(x, partner)
    return x


def _kernel(xT_hbm, mem0_ref, wq_hbm, wk_hbm, wv_hbm, woT_hbm, wr_ref, wg_hbm, wu_hbm,
            wdT_hbm, c_ref, wmod_hbm, out_hbm,
            xT, wq, wk, wv, woT, wg, wu, wdT, wmod, ab, cols, hs, ao, cur, late, outv, selbuf,
            sems):
    halves = [
        [pltpu.make_async_copy(src.at[:, pl.ds(e * 128, 128)], dst.at[e], sems.at[10 + 2 * n + e])
         for e in range(2)]
        for n, (src, dst) in enumerate(
            [(wq_hbm, wq), (wk_hbm, wk), (woT_hbm, woT), (wv_hbm, wv)])]
    for pair in halves:
        for cp in pair:
            cp.start()
    copies = [
        None, None, None, None,
        pltpu.make_async_copy(wmod_hbm, wmod, sems.at[4]),
        pltpu.make_async_copy(xT_hbm, xT, sems.at[5]),
        pltpu.make_async_copy(wg_hbm, wg, sems.at[6]),
        pltpu.make_async_copy(wu_hbm, wu, sems.at[7]),
        pltpu.make_async_copy(wdT_hbm, wdT, sems.at[8]),
    ]
    for cp in copies[4:]:
        cp.start()

    lane448 = lax.broadcasted_iota(jnp.int32, (D, 128), 1)

    def head_pair(w_ref, p):
        w32 = jnp.concatenate(
            [w_ref.bitcast(U32)[e, pl.ds(p, D, stride=H // 2), :] for e in range(2)], axis=1)
        even = pltpu.bitcast(w32 << 16, F32).astype(BF16)
        odd = pltpu.bitcast(w32 & jnp.uint32(0xFFFF0000), F32).astype(BF16)
        return even, odd

    def fold(base, p, lhs_e, lhs_o, rhs_e, rhs_o, scale):
        me = _dot_nt(lhs_e, _dup_rows(rhs_e))
        mo = _dot_nt(lhs_o, _dup_rows(rhs_o))
        if scale is not None:
            me = me * scale
            mo = mo * scale
        for j in range(3):
            c0 = base + j * H + 2 * p
            ab[c0] = _pack(me[:, j * 128:(j + 1) * 128])
            ab[c0 + 1] = _pack(mo[:, j * 128:(j + 1) * 128])
        ab[base + 3 * H + p] = _pack(jnp.where(lane448 < 64, me[:, 384:], mo[:, 384:]))

    for cp in halves[0] + halves[1]:
        cp.wait()
    for p in range(H // 2):
        qe, qo = head_pair(wq, p)
        ke, ko = head_pair(wk, p)
        fold(0, p, ke, ko, qe, qo, E ** -0.5)
    for cp in halves[2] + halves[3]:
        cp.wait()

    def wo_head(h):
        return jnp.concatenate([woT[e, h * D:(h + 1) * D, :] for e in range(2)], axis=1)

    for p in range(H // 2):
        ve, vo = head_pair(wv, p)
        fold(HALF, p, ve, vo, wo_head(2 * p), wo_head(2 * p + 1), None)

    copies[4].wait()
    c = c_ref[...].astype(F32)
    sc = c * (1.0 / (1.0 + jnp.exp(-c)))
    mod = _round_bf16(_dot(jnp.broadcast_to(sc, (16, D)).astype(BF16), wmod[...]))
    modT = jnp.broadcast_to(mod[0:1], (128, 6 * D)).T
    cols[0] = modT[0 * D:1 * D]
    cols[1] = _round_bf16(1.0 + modT[1 * D:2 * D])
    cols[2] = modT[2 * D:3 * D]
    cols[3] = modT[3 * D:4 * D]
    cols[4] = _round_bf16(1.0 + modT[4 * D:5 * D])
    cols[5] = modT[5 * D:6 * D]
    wr = wr_ref[...].astype(F32).reshape(1, D)
    wr = jnp.concatenate([wr, jnp.zeros((1, DP - D), F32)], axis=1)
    cols[6] = jnp.broadcast_to(wr, (128, DP)).T[:D]

    def layernorm(x):
        m = jnp.mean(x, axis=0, keepdims=True)
        d = x - m
        v = jnp.mean(d * d, axis=0, keepdims=True)
        return d * (1.0 / jnp.sqrt(v + 1e-5))

    def modulate(g):
        t0 = pl.multiple_of(g * G, G)
        x = xT[:, pl.ds(t0, G)].astype(F32)
        h = layernorm(x) * cols[1] + cols[0]
        hs[pl.ds(t0, G), :] = _dup_rows(h).T

    def residual(g):
        t0 = pl.multiple_of(g * G, G)
        a = ao[pl.ds(t0, G), :].T[:D]
        x1 = xT[:, pl.ds(t0, G)].astype(F32) + cols[2] * a
        h2 = layernorm(x1) * cols[4] + cols[3]
        return t0, x1, h2

    lane1 = lax.broadcasted_iota(jnp.int32, (1, 128), 1)

    def finish(g, best, best_idx):
        t0, x1, h2 = residual(g)
        r = _round_bf16(jnp.sum(h2 * cols[6], axis=0, keepdims=True))
        outv[:, pl.ds(t0, G)] = (x1 + cols[5] * (h2 + h2 * 0.0)).astype(BF16)
        better = r > best
        return jnp.where(better, r, best), jnp.where(better, lane1 + t0, best_idx)

    lane8 = lax.broadcasted_iota(jnp.int32, (8, 128), 1)
    lane40 = lax.broadcasted_iota(jnp.int32, (M + SEG, 128), 1)
    row40 = lax.broadcasted_iota(jnp.int32, (M + SEG, 128), 0)

    def weights(tiles):
        return jnp.concatenate([_unpack(ab[t]) for t in tiles], axis=1)

    def heads4(o, i):
        return _pack(jnp.concatenate(
            [o[8 * i:8 * i + 8, 128 * q:128 * q + 128] for q in range(4)], axis=0))

    def pairs(o, i, qs):
        parts = []
        for q in qs:
            x = o[8 * i:8 * i + 8, 128 * q:128 * q + 128]
            parts.append(jnp.where(lane8 < 64, x, 0.0))
            parts.append(jnp.where(lane8 < 64, 0.0, x))
        return _pack(jnp.concatenate(parts, axis=0))

    def project(lhs, kv, chunk):
        if chunk < 12:
            j, cq = divmod(chunk, 4)
            o = _dot(lhs, weights([kv * HALF + j * H + 4 * cq + q for q in range(4)]))
            for t in range(4):
                cur[kv, j, t * 64 + 16 * cq:t * 64 + 16 * cq + 16, :] = heads4(o, t)
        else:
            cq = chunk - 12
            o = _dot(lhs, weights([kv * HALF + 3 * H + 4 * cq + q for q in range(4)]))
            for t in range(4):
                cur[kv, 3, t * 64 + 32 * cq:t * 64 + 32 * cq + 32, :] = pairs(o, t, range(4))

    def project_late(lhs, par, cq, chunk):
        if chunk < 6:
            kv, j = divmod(chunk, 3)
            o = _dot(lhs, weights([kv * HALF + j * H + 4 * cq + q for q in range(4)]))
            for i in range(4):
                late[par, i, kv, j, 16 * cq:16 * cq + 16, :] = heads4(o, i)
        else:
            o = _dot(lhs, weights([kv * HALF + 3 * H + 2 * cq + q
                                   for kv in range(2) for q in range(2)]))
            for i in range(4):
                for kv in range(2):
                    late[par, i, kv, 3, 16 * cq:16 * cq + 16, :] = pairs(
                        o, i, (2 * kv, 2 * kv + 1))

    def late_rows(g):
        t0 = pl.multiple_of(g * G, G)
        rows = [hs[pl.ds(t0 + SEG * i + 24, 8), :] for i in range(4)]
        return jnp.concatenate(rows, axis=0).astype(BF16)[:, :D]

    def stationary(kv, par, i):
        return jnp.concatenate(
            [_unpack(jnp.concatenate([cur[kv, j], late[par, i, kv, j]], axis=0))
             for j in range(4)], axis=1)

    def softmax(s):
        ss = []
        for t in range(5):
            st = s[:M + SEG, t * 128:(t + 1) * 128]
            if t > 0:
                allowed = (row40 < M) | (row40 >= 8 * t + (lane40 & 7))
                st = jnp.where(allowed, st, NEG)
            ss.append(st)
        mx = _group8(functools.reduce(jnp.maximum, ss), jnp.maximum, lane40)
        es = [jnp.exp(st - mx) for st in ss]
        inv = 1.0 / _group8(functools.reduce(jnp.add, es), jnp.add, lane40)
        p = jnp.concatenate([e * inv for e in es], axis=1)
        return jnp.concatenate([p, jnp.zeros((8, 640), F32)], axis=0).astype(BF16)

    def segment(g, i, mem, ahead):
        par = g & 1
        t0 = pl.multiple_of(g * G + SEG * i, SEG)
        rows = jnp.concatenate([mem, hs[pl.ds(t0, SEG), :], mem], axis=0).astype(BF16)
        lhs = rows[:32, :D]
        for chunk in range(14):
            project(lhs, 0, chunk)
        for chunk in range(2):
            project(lhs, 1, chunk)
        s = _dot_nt(rows, stationary(0, par, i))
        for chunk in range(2, 14):
            project(lhs, 1, chunk)
        p = softmax(s)
        for chunk in range(2):
            project_late(ahead, 1 - par, i, chunk)
        o = _dot(p, stationary(1, par, i))[:M + SEG]
        for chunk in range(2, 7):
            project_late(ahead, 1 - par, i, chunk)
        tail = o[:, 384:]
        tail = tail + pltpu.roll(tail, 64, 1)
        o = jnp.concatenate([o[:, :384], tail], axis=1)
        ao[pl.ds(t0, SEG), :] = o[M:]
        return o[:M]

    copies[5].wait()
    modulate(0)
    modulate(1)
    first = late_rows(0)
    for cq in range(4):
        for chunk in range(7):
            project_late(first, 0, cq, chunk)
    ao[0:G, :] = jnp.zeros((G, DP), F32)

    def group(g, carry):
        mem, best, best_idx = carry
        ahead = late_rows(jnp.minimum(g + 1, NG - 1))
        prev = jnp.maximum(g - 1, 0)
        b, bi = finish(prev, best, best_idx)
        best = jnp.where(g > 0, b, best)
        best_idx = jnp.where(g > 0, bi, best_idx)
        for i in range(4):
            mem = segment(g, i, mem, ahead)
            if i == 1:
                modulate(jnp.minimum(g + 2, NG - 1))
        return mem, best, best_idx

    mem0 = mem0_ref[...].astype(F32)
    mem0 = jnp.concatenate([mem0, mem0[:, 384:448]], axis=1)
    _, best, best_idx = lax.fori_loop(
        0, NG, group,
        (mem0, jnp.full((1, 128), -jnp.inf, F32), jnp.zeros((1, 128), jnp.int32)))
    best, best_idx = finish(NG - 1, best, best_idx)
    r_sel = jnp.max(best, axis=1, keepdims=True)
    idx = jnp.min(jnp.where(best == r_sel, best_idx, S - 1))
    idx = jnp.clip(idx, 0, S - 1)

    col = idx % G
    t0, x1, h2 = residual(idx // G)
    selbuf[...] = _dup_rows(h2).T
    x_sel = jnp.broadcast_to(selbuf[pl.ds(col, 1), :], (16, DP))[:, :D].astype(BF16)
    copies[6].wait()
    copies[7].wait()
    gate = _dot(x_sel, wg[...])
    up = _dot(x_sel, wu[...])
    act = (gate * (1.0 / (1.0 + jnp.exp(-gate))) * up).astype(BF16)
    copies[8].wait()
    y = _dot_nt(act, _dup_rows(wdT[...]))[0:1]
    y = y * (1.0 / (1.0 + jnp.exp(-r_sel)))
    yT = jnp.broadcast_to(y, (128, DP)).T[:D]
    upd = jnp.where(lane448 == col, yT, 0.0)
    outv[:, pl.ds(t0, G)] = (x1 + cols[5] * (h2 + (h2 * 0.0 + upd))).astype(BF16)

    out_copy = pltpu.make_async_copy(outv, out_hbm, sems.at[9])
    out_copy.start()
    out_copy.wait()


@jax.jit
def pallas_adaLN_cond__memory_aug_recurrent_mem_tr__moe_arch_mod__prompt_kernel(
        A_x, A_mem0, A_Wq, A_Wk, A_Wv, A_Wo, A_seg_len, B_x, B_w_r, B_w_gate, B_w_up,
           B_w_down, c, w_mod):
    del A_seg_len, B_x
    xT = A_x.reshape(S, D).T
    hbm = pl.BlockSpec(memory_space=pl.ANY)
    vmem = pl.BlockSpec(memory_space=pltpu.VMEM)
    outT = pl.pallas_call(
        _kernel,
        out_shape=jax.ShapeDtypeStruct((D, S), BF16),
        in_specs=[hbm, vmem, hbm, hbm, hbm, hbm, vmem, hbm, hbm, hbm, vmem, hbm],
        out_specs=hbm,
        scratch_shapes=[
            pltpu.VMEM((D, S), BF16),
            pltpu.VMEM((2, D * H, 128), BF16),
            pltpu.VMEM((2, D * H, 128), BF16),
            pltpu.VMEM((2, D * H, 128), BF16),
            pltpu.VMEM((2, H * D, 128), BF16),
            pltpu.VMEM((D, F), BF16),
            pltpu.VMEM((D, F), BF16),
            pltpu.VMEM((D, F), BF16),
            pltpu.VMEM((D, 6 * D), BF16),
            pltpu.VMEM((2 * HALF, D // 2, 128), U32),
            pltpu.VMEM((7, D, 128), F32),
            pltpu.VMEM((S, DP), F32),
            pltpu.VMEM((S, DP), F32),
            pltpu.VMEM((2, 4, 256, 128), U32),
            pltpu.VMEM((2, 4, 2, 4, 64, 128), U32),
            pltpu.VMEM((D, S), BF16),
            pltpu.VMEM((128, DP), F32),
            pltpu.SemaphoreType.DMA((18,)),
        ],
        compiler_params=pltpu.CompilerParams(vmem_limit_bytes=100 * 1024 * 1024),
        name="adaln_rmt_mod",
    )(xT, A_mem0.reshape(M, D), A_Wq.reshape(D * H, E), A_Wk.reshape(D * H, E),
      A_Wv.reshape(D * H, E), A_Wo.transpose(0, 2, 1).reshape(H * D, E), B_w_r, B_w_gate,
      B_w_up, B_w_down.T, c, w_mod)
    return outT.T.reshape(1, S, D)
```

```python
import functools

import jax
import jax.numpy as jnp
import numpy as np
from jax import lax
import jax.experimental.pallas as pl
import jax.experimental.pallas.tpu as pltpu

F32 = jnp.float32
BF16 = jnp.bfloat16
U32 = jnp.uint32

D = 448
DM = 384
DP = 512
H = 16
E = 256
M = 8
SEG = 32
S = 2048
F = 1792
G = 128
NG = S // G
HALF = H * D // 128
MASKED = -1000000000.0
EPS = 1e-5

K_ROWS = ((0, 128), (128, 320))
V_ROWS = ((0, 256), (256, 192))
O_PAIRS = ((0, 2), (2, 3), (5, 3))
N_COPIES = 2 * (1 + len(K_ROWS) + len(V_ROWS) + len(O_PAIRS)) + 9
FEATURE_BLOCKS = ((0, 128), (128, 128), (256, 128), (384, 64))
SIDE_STEPS = ((1, 3, 5, 7, 9, 11), (1, 3, 5, 7), (1,), (1, 3, 5, 7))
LONG_CHUNKS = 2


def _dot(a, b):
    return lax.dot_general(a, b, (((1,), (0,)), ((), ())), preferred_element_type=F32)


def _dot_nt(a, b):
    return lax.dot_general(a, b, (((1,), (1,)), ((), ())), preferred_element_type=F32)


def _round_bf16(x):
    return x.astype(BF16).astype(F32)


def _pack(x):
    return pltpu.bitcast(x.astype(BF16), U32)


def _unpack(x):
    return pltpu.bitcast(x, BF16)


def _dup_rows(w):
    return jnp.concatenate([w, w[DM:D]], axis=0)


def _sigmoid(x):
    return 1.0 / (1.0 + jnp.exp(-x))


def _fold8(x):
    return functools.reduce(jnp.add, [x[r:r + 8] for r in range(0, x.shape[0], 8)])


def _mean(acc):
    return jnp.sum(acc, axis=0, keepdims=True) * (1.0 / D)


def _inv_std(acc):
    return 1.0 / jnp.sqrt(_mean(acc) + EPS)


def _group8(x, op, lane):
    for s in (1, 2, 4):
        partner = jnp.where((lane & s) == 0, pltpu.roll(x, 128 - s, 1), pltpu.roll(x, s, 1))
        x = op(x, partner)
    return x


def _start_of(index, size):
    return index * size if isinstance(index, int) else pl.multiple_of(index * size, size)


def _run(task):
    for _ in task:
        pass


def _wait(copies):
    for copy in copies:
        copy.wait()


def _kernel(xT_hbm, mem0_hbm, wq_hbm, wk_hbm, wv_hbm, woT_hbm, wr_hbm, wg_hbm, wu_hbm,
            wdT_hbm, c_hbm, wmod_hbm, out_hbm,
            xT, mem0, wqs, wks, wvs, wos, wq_heads, part, part_tail, wr, wg, wu, wdT, c, wmod,
            ab, qtail, vtail, cols, hs, ao, cur, late, late_q, outv, h2s, sems, out_sems):
    started = []

    def start(src, dst):
        copy = pltpu.make_async_copy(src, dst, sems.at[len(started)])
        started.append(copy)
        copy.start()
        return [copy]

    def start_half(src, r0, n, e, dst):
        return start(src.at[pl.ds(r0, n), pl.ds(e * 128, 128)], dst.at[pl.ds(0, n)])

    def start_tokens(t0, n):
        return start(xT_hbm.at[:, pl.ds(t0, n)], xT.at[:, pl.ds(t0, n)])

    def start_values(ci):
        r0, n = V_ROWS[ci]
        return sum((start_half(wv_hbm, r0 * H, n * H, e, wvs[ci][e]) for e in range(2)), [])

    cp_q, cp_k = [], []
    for e in range(2):
        cp_q.append(start_half(wq_hbm, 0, D * H, e, wqs[e]))
        cp_k.append([start_half(wk_hbm, r0 * H, n * H, e, buf)
                     for (r0, n), buf in zip(K_ROWS, wks[e])])
    cp_v = [start_values(0)]
    cp_o = [sum((start_half(woT_hbm, 2 * p0 * D, 2 * n * D, e, buf[e]) for e in range(2)), [])
            for (p0, n), buf in zip(O_PAIRS, wos)]
    cp_v.append(start_values(1))
    cp_small = (start(c_hbm, c) + start(mem0_hbm, mem0) + start(wr_hbm, wr)
                + start(wmod_hbm, wmod) + start_tokens(0, 2 * G))
    cp_tokens = start_tokens(2 * G, S - 2 * G)
    cp_ffn = start(wg_hbm, wg) + start(wu_hbm, wu) + start(wdT_hbm, wdT)

    def head_pair(w_ref, p, n):
        w32 = w_ref.bitcast(U32)[pl.ds(p, n, stride=H // 2), :]
        even = pltpu.bitcast(w32 << 16, F32).astype(BF16)
        odd = pltpu.bitcast(w32 & np.uint32(0xFFFF0000), F32).astype(BF16)
        return even, odd

    def fold(lhs, rhs):
        pad = -lhs[0].shape[0] % 128
        main = [_dot_nt(l, r[:DM]) for l, r in zip(lhs, rhs)]
        tail = [_dot_nt(r[DM:], jnp.concatenate([l, l[:pad]], axis=0) if pad else l)
                for l, r in zip(lhs, rhs)]
        return main + [jnp.concatenate(tail, axis=0)]

    def store_folded(kv, p, r0, even, odd, tail):
        n = even.shape[0]
        m = min(n, DM - r0)
        tail = tail.T[:n]
        rows = slice(r0 // 2, (r0 + m) // 2)
        for j in range(3):
            c0 = kv * HALF + j * H + 2 * p
            ab[c0, rows] = _pack(even[:m, j * 128:(j + 1) * 128])
            ab[c0 + 1, rows] = _pack(odd[:m, j * 128:(j + 1) * 128])
        ab[kv * HALF + 3 * H + p, rows] = _pack(tail[:m])
        if m == n:
            return
        if kv == 0:
            corner = jnp.concatenate([tail[m:], pltpu.roll(tail[m:], 64, 1)], axis=0)
            both = jnp.concatenate([jnp.concatenate([even[m:], odd[m:]], axis=0), corner], axis=1)
            qtail[p] = _pack(both.T[:D])
            return
        for j in range(3):
            vtail[j, 64 * p:64 * p + 64] = _pack(jnp.concatenate(
                [even[m:, j * 128:(j + 1) * 128], odd[m:, j * 128:(j + 1) * 128]], axis=0))
        left = lax.broadcasted_iota(jnp.int32, (D - DM, 128), 1) < 64
        vtail[3, 64 * p:64 * p + 64] = _pack(jnp.concatenate(
            [jnp.where(left, tail[m:], 0.0), jnp.where(left, 0.0, tail[m:])], axis=0))

    for e in range(2):
        _wait(cp_q[e])
        for ci, (r0, n) in enumerate(K_ROWS):
            _wait(cp_k[e][ci])
            for p in range(H // 2):
                if ci == 0:
                    rhs = head_pair(wqs[e], p, D)
                    for odd in range(2):
                        wq_heads[2 * p + odd] = pltpu.bitcast(rhs[odd], U32)
                else:
                    rhs = [_unpack(wq_heads[2 * p + odd]) for odd in range(2)]
                ms = fold(head_pair(wks[e][ci], p, n), rhs)
                slots = [part.at[2 * p, r0:r0 + n], part.at[2 * p + 1, r0:r0 + n],
                         part_tail.at[ci, p, :, :ms[2].shape[1]]]
                if e == 0:
                    for slot, x in zip(slots, ms):
                        slot[...] = x
                else:
                    store_folded(0, p, r0, *(
                        (slot[...] + x) * E ** -0.5 for slot, x in zip(slots, ms)))

    for ci, (r0, n) in enumerate(V_ROWS):
        _wait(cp_v[ci])
        for (p0, count), buf, copies in zip(O_PAIRS, wos, cp_o):
            if ci == 0:
                _wait(copies)
            for p in range(count):
                lhs = [head_pair(wvs[ci][e], p0 + p, n) for e in range(2)]
                lhs = [jnp.concatenate([lhs[e][odd] for e in range(2)], axis=1)
                       for odd in range(2)]
                rhs = [jnp.concatenate([buf[e][h * D:(h + 1) * D, :] for e in range(2)], axis=1)
                       for h in (2 * p, 2 * p + 1)]
                store_folded(1, p0 + p, r0, *fold(lhs, rhs))

    _wait(cp_small)
    cond = c[...].astype(F32)
    mod = _round_bf16(_dot(jnp.broadcast_to(cond * _sigmoid(cond), (8, D)), wmod[...]))
    mod = jnp.broadcast_to(mod[0:1], (128, 6 * D)).T
    for n in range(6):
        col = mod[n * D:(n + 1) * D]
        cols[n] = _round_bf16(1.0 + col) if n % 3 == 1 else col
    router = jnp.concatenate(
        [wr[...].astype(F32).reshape(1, D), jnp.zeros((1, DP - D), F32)], axis=1)
    cols[6] = jnp.broadcast_to(router, (128, DP)).T[:D]

    SUM, SQ, SCORE, SQ2 = (pl.ds(D + 8 * n, 8) for n in range(4))

    def modulate(g):
        t = pl.ds(_start_of(g, G), G)
        hs[4, SUM, :] = sum(_fold8(xT[r:r + n, t].astype(F32)) for r, n in FEATURE_BLOCKS)
        yield
        m = _mean(hs[4, SUM, :])
        ds = [xT[r:r + n, t].astype(F32) - m for r, n in FEATURE_BLOCKS]
        hs[4, SQ, :] = sum(_fold8(d * d) for d in ds)
        yield
        inv = _inv_std(hs[4, SQ, :])
        for j, (r, n) in enumerate(FEATURE_BLOCKS):
            h = (xT[r:r + n, t].astype(F32) - m) * inv * cols[1, r:r + n] + cols[0, r:r + n]
            if n < 128:
                h = jnp.concatenate([h, h], axis=0)
            hs[j, t, :] = h.T
            yield

    def finish(g, scores):
        t = pl.ds(_start_of(g, G), G)
        acc = jnp.zeros((8, 128), F32)
        for j, (r, n) in enumerate(FEATURE_BLOCKS):
            a = ao[t, 128 * j:128 * j + 128].T[:n]
            x1 = xT[r:r + n, t].astype(F32) + cols[2, r:r + n] * a
            hs[4, r:r + n, :] = x1
            acc = acc + _fold8(x1)
            yield
        m = _mean(acc)
        ds = [hs[4, r:r + n, :] - m for r, n in FEATURE_BLOCKS]
        hs[4, SQ2, :] = sum(_fold8(d * d) for d in ds)
        yield
        inv = _inv_std(hs[4, SQ2, :])
        acc = jnp.zeros((8, 128), F32)
        for r, n in FEATURE_BLOCKS:
            x1 = hs[4, r:r + n, :]
            h2 = (x1 - m) * inv * cols[4, r:r + n] + cols[3, r:r + n]
            hs[4, SCORE, :] = acc + _fold8(h2 * cols[6, r:r + n])
            outv[r:r + n, t] = (x1 + cols[5, r:r + n] * (h2 + h2 * 0.0)).astype(BF16)
            h2s[g, r // 2:(r + n) // 2] = _pack(h2)
            yield
            acc = hs[4, SCORE, :]
        scores.append(_round_bf16(jnp.sum(acc, axis=0, keepdims=True)))

    lane1 = lax.broadcasted_iota(jnp.int32, (1, 128), 1)

    def better(r, g, best, best_idx):
        take = (r > best) & (g >= 0)
        return jnp.where(take, r, best), jnp.where(take, lane1 + g * G, best_idx)

    lane8 = lax.broadcasted_iota(jnp.int32, (8, 128), 1)
    lane40 = lax.broadcasted_iota(jnp.int32, (M + SEG, 128), 1)
    row40 = lax.broadcasted_iota(jnp.int32, (M + SEG, 128), 0)

    def weights(ref, tiles):
        return jnp.concatenate([_unpack(ref[t]) for t in tiles], axis=1)

    def heads4(o, i):
        return _pack(jnp.concatenate(
            [o[8 * i:8 * i + 8, 128 * q:128 * q + 128] for q in range(4)], axis=0))

    def pairs(o, i, qs):
        parts = []
        for q in qs:
            x = o[8 * i:8 * i + 8, 128 * q:128 * q + 128]
            parts.append(jnp.where(lane8 < 64, x, 0.0))
            parts.append(jnp.where(lane8 < 64, 0.0, x))
        return _pack(jnp.concatenate(parts, axis=0))

    def keep(o, kv, chunk):
        j, cq = divmod(chunk, 4)
        n = 16 if j < 3 else 32
        for t in range(4):
            cur[kv, j, 64 * t + n * cq:64 * t + n * (cq + 1), :] = (
                heads4(o, t) if j < 3 else pairs(o, t, range(4)))

    def keep_late(o, par, kv, j, cq):
        for i in range(4):
            late[par, i, kv, j, 16 * cq:16 * cq + 16, :] = heads4(o, i)

    def project(lhs, kv, chunk):
        keep(_dot(lhs[:, :DM], weights(ab, [kv * HALF + 4 * chunk + q for q in range(4)])),
             kv, chunk)

    def project_late(lhs, par, cq, chunk):
        if chunk < 6:
            kv, j = divmod(chunk, 3)
            o = _dot(lhs[:, :DM], weights(ab, [kv * HALF + j * H + 4 * cq + q for q in range(4)]))
            keep_late(o, par, kv, j, cq)
        else:
            o = _dot(lhs[:, :DM], weights(ab, [kv * HALF + 3 * H + 2 * cq + q
                                               for kv in range(2) for q in range(2)]))
            for i in range(4):
                for kv in range(2):
                    late[par, i, kv, 3, 16 * cq:16 * cq + 16, :] = pairs(
                        o, i, (2 * kv, 2 * kv + 1))

    def project_both(lhs, par, kv, j, cq):
        o = None
        for k in range(3):
            w = jnp.concatenate(
                [_unpack(ab[kv * HALF + j * H + 4 * cq + q, 64 * k:64 * k + 64]) for q in range(4)],
                axis=1)
            x = _dot(lhs[:, 128 * k:128 * k + 128], w)
            o = x if o is None else o + x
            if k == 2:
                keep(o[:32], kv, 4 * j + cq)
                keep_late(o[32:], par, kv, j, cq)
            yield

    def project_queries(lhs, half):
        return _dot(lhs, weights(qtail, range(4 * half, 4 * half + 4)))

    def token_rows(t0, n):
        return jnp.concatenate([hs[j, pl.ds(t0, n), :] for j in range(4)], axis=1)

    def late_rows(g):
        t0 = _start_of(g, G)
        rows = [token_rows(t0 + SEG * i + 24, 8) for i in range(4)]
        return jnp.concatenate(rows, axis=0).astype(BF16)[:, :D]

    def segment(g, i, mem, ahead, side):
        par = g & 1
        t0 = _start_of(4 * g + i, SEG)
        rows = jnp.concatenate([mem, token_rows(t0, SEG)], axis=0)
        lhs = rows[:32].astype(BF16)[:, :D]
        slot = lane40 >> 4
        tails = [pairs(rows, t, (3,)) for t in range(5)] + [jnp.zeros((8, 128), U32)] * 3
        zs = [_unpack(jnp.concatenate([tails[(u - p) % 8] for u in range(8)], axis=0))
              for p in range(8)]
        both = jnp.concatenate([lhs, ahead], axis=0)
        for chunk in range(14):
            if chunk == 6:
                q = jnp.concatenate([project_queries(lhs, half) for half in range(2)], axis=1)
                q = jnp.concatenate([q, late_q[par, 8 * i:8 * i + 8, :]], axis=0)
            project(lhs, 0, chunk)
            if chunk in SIDE_STEPS[i]:
                next(side, None)

        def long_passes():
            for j in range(LONG_CHUNKS):
                yield from project_both(both, 1 - par, 1, j, i)

        cover = long_passes()
        next(cover, None)
        raw = []
        for p in range(8):
            raw.append(_dot_nt(q[:, 128 * p:128 * p + 128], zs[p]))
            if p % 4 == 3:
                next(cover, None)
        s = None
        for j in range(4):
            x = _dot_nt(rows[:, 128 * j:128 * j + 128], _unpack(cur[0, j]))
            s = x if s is None else s + x
            next(cover, None)
        s = jnp.concatenate([s, _dot_nt(rows, weights(late.at[par, i, 0], range(4)))], axis=1)
        _run(cover)
        for chunk in range(14):
            if chunk not in [4 * j + i for j in range(LONG_CHUNKS)]:
                project(lhs, 1, chunk)

        ss = []
        for t in range(5):
            x = raw[0]
            for p in range(1, 8):
                x = jnp.where(slot == (p + t) % 8, raw[p], x)
            if t > 0:
                x = pltpu.roll(x, 128 - 16 * t, 1)
            st = s[:, t * 128:(t + 1) * 128] + x
            if t > 0:
                allowed = (row40 < M) | (row40 >= 8 * t + (lane40 & 7))
                st = jnp.where(allowed, st, MASKED)
            ss.append(st)
        mx = _group8(functools.reduce(jnp.maximum, ss), jnp.maximum, lane40)
        es = [jnp.exp(st - mx) for st in ss]
        inv = 1.0 / _group8(functools.reduce(jnp.add, es), jnp.add, lane40)
        ps = [e * inv for e in es]

        ys = [ps[0]] + [pltpu.roll(ps[t], 16 * t, 1) for t in range(1, 5)]
        z = []
        for p in range(8):
            x = ys[0]
            for t in range(1, 5):
                x = jnp.where(slot == (p + t) % 8, ys[t], x)
            z.append(_dot(x, zs[p]))
        values = jnp.concatenate(
            [_unpack(jnp.concatenate([cur[1, j], late[par, i, 1, j]], axis=0)) for j in range(4)],
            axis=1)
        o = (_dot(jnp.concatenate(z, axis=1), weights(vtail, range(4)))
             + _dot(jnp.concatenate(ps, axis=1), values))
        for chunk in range(7):
            if not 3 <= chunk < 3 + LONG_CHUNKS:
                project_late(ahead, 1 - par, i, chunk)
        if i % 2 == 0:
            late_q[1 - par, :, 256 * i:256 * i + 512] = project_queries(ahead, i // 2)
        tail = o[:, DM:]
        o = jnp.concatenate([o[:, :DM], tail + pltpu.roll(tail, 64, 1)], axis=1)
        ao[pl.ds(t0, SEG), :] = o[M:]
        return o[:M]

    _run(modulate(0))
    _run(modulate(1))
    first = late_rows(0)
    for half in range(2):
        late_q[0, :, 512 * half:512 * half + 512] = project_queries(first, half)
    for cq in range(4):
        for chunk in range(7):
            project_late(first, 0, cq, chunk)
    ao[0:G, :] = jnp.zeros((G, DP), F32)
    _wait(cp_tokens)

    def out_copy(g, count, sem):
        t = pl.ds(_start_of(g, G), count * G)
        return pltpu.make_async_copy(outv.at[:, t], out_hbm.at[:, t], out_sems.at[sem])

    cp_out = [out_copy(0, NG - 2, 0), out_copy(NG - 2, 2, 1)]

    def group(g, carry):
        mem, best, best_idx = carry

        @pl.when(g == NG - 1)
        def _():
            cp_out[0].start()

        ahead = late_rows(jnp.minimum(g + 1, NG - 1))
        scores = []

        def side_work():
            yield from modulate(jnp.minimum(g + 2, NG - 1))
            yield from finish(jnp.maximum(g - 1, 0), scores)

        side = side_work()
        for i in range(4):
            mem = segment(g, i, mem, ahead, side)
        _run(side)
        return (mem,) + better(scores[0], g - 1, best, best_idx)

    mem = mem0[...].astype(F32)
    mem = jnp.concatenate([mem, mem[:, DM:D]], axis=1)
    _, best, best_idx = lax.fori_loop(
        0, NG, group, (mem, jnp.full((1, 128), -jnp.inf, F32), jnp.zeros((1, 128), jnp.int32)))
    scores = []
    _run(finish(NG - 1, scores))
    best, best_idx = better(scores[0], NG - 1, best, best_idx)
    cp_out[1].start()

    r_sel = jnp.max(best, axis=1, keepdims=True)
    idx = jnp.clip(jnp.min(jnp.where(best == r_sel, best_idx, S - 1)), 0, S - 1)
    g_sel, col = idx // G, idx % G
    pick = (lax.broadcasted_iota(jnp.int32, (8, G), 1) == col).astype(F32)
    x_sel = _dot_nt(pick, _dup_rows(_unpack(h2s[g_sel])))[:, :D]
    _wait(cp_ffn)
    gate = _dot(x_sel, wg[...])
    up = _dot(x_sel, wu[...])
    y = _dot_nt(gate * _sigmoid(gate) * up, _dup_rows(wdT[...]))[0:1] * _sigmoid(r_sel)
    y = jnp.broadcast_to(y, (128, DP)).T[:D]
    update = jnp.where(lax.broadcasted_iota(jnp.int32, (D, 128), 1) == col, y, 0.0)
    _wait(cp_out)
    t = pl.ds(_start_of(g_sel, G), G)
    outv[:, t] = (outv[:, t].astype(F32) + cols[5] * update).astype(BF16)
    last = out_copy(g_sel, 1, 2)
    last.start()
    last.wait()


@jax.jit
def pallas_adaLN_cond__memory_aug_recurrent_mem_tr__moe_arch_mod__prompt_kernel(
        A_x, A_mem0, A_Wq, A_Wk, A_Wv, A_Wo, A_seg_len, B_x, B_w_r, B_w_gate, B_w_up,
           B_w_down, c, w_mod):
    del A_seg_len, B_x
    hbm = pl.BlockSpec(memory_space=pl.ANY)

    def feature_rows(n):
        return pltpu.VMEM(((n + 1) * H, 128), BF16)

    outT = pl.pallas_call(
        _kernel,
        out_shape=jax.ShapeDtypeStruct((D, S), BF16),
        in_specs=[hbm] * 12,
        out_specs=hbm,
        scratch_shapes=[
            pltpu.VMEM((D, S), BF16),
            pltpu.VMEM((M, D), BF16),
            [feature_rows(D)] * 2,
            [[feature_rows(n) for _, n in K_ROWS]] * 2,
            [[feature_rows(n)] * 2 for _, n in V_ROWS],
            [[pltpu.VMEM((2 * n * D, 128), BF16)] * 2 for _, n in O_PAIRS],
            pltpu.VMEM((H, D // 2, 128), U32),
            pltpu.VMEM((H, D, DM), F32),
            pltpu.VMEM((len(K_ROWS), H // 2, 128, DM), F32),
            pltpu.VMEM((D,), BF16),
            pltpu.VMEM((D, F), BF16),
            pltpu.VMEM((D, F), BF16),
            pltpu.VMEM((D, F), BF16),
            pltpu.VMEM((1, D), BF16),
            pltpu.VMEM((D, 6 * D), BF16),
            pltpu.VMEM((2 * HALF, DM // 2, 128), U32),
            pltpu.VMEM((H // 2, D // 2, 128), U32),
            pltpu.VMEM((4, H * 32, 128), U32),
            pltpu.VMEM((7, D, 128), F32),
            pltpu.VMEM((5, S, 128), F32),
            pltpu.VMEM((S, DP), F32),
            pltpu.VMEM((2, 4, 256, 128), U32),
            pltpu.VMEM((2, 4, 2, 4, 64, 128), U32),
            pltpu.VMEM((2, 32, 1024), F32),
            pltpu.VMEM((D, S), BF16),
            pltpu.VMEM((NG, D // 2, G), U32),
            pltpu.SemaphoreType.DMA((N_COPIES,)),
            pltpu.SemaphoreType.DMA((3,)),
        ],
        compiler_params=pltpu.CompilerParams(vmem_limit_bytes=100 * 1024 * 1024),
        name="adaln_rmt_mod",
    )(A_x.reshape(S, D).T, A_mem0.reshape(M, D), A_Wq.reshape(D * H, E), A_Wk.reshape(D * H, E),
      A_Wv.reshape(D * H, E), A_Wo.transpose(0, 2, 1).reshape(H * D, E), B_w_r, B_w_gate,
      B_w_up, B_w_down.T, c, w_mod)
    return outT.T.reshape(1, S, D)
```

```python
import functools

import jax
import jax.numpy as jnp
import numpy as np
from jax import lax
import jax.experimental.pallas as pl
import jax.experimental.pallas.tpu as pltpu

F32 = jnp.float32
BF16 = jnp.bfloat16
U32 = jnp.uint32

D = 448
DM = 384
DP = 512
H = 16
E = 256
M = 8
SEG = 32
S = 2048
F = 1792
G = 128
NG = S // G
HALF = H * D // 128
MASKED = -1000000000.0
EPS = 1e-5

K_ROWS = ((0, 128), (128, 320))
V_ROWS = ((0, 256), (256, 192))
O_PAIRS = ((0, 2), (2, 3), (5, 3))
N_COPIES = 2 * (1 + len(K_ROWS) + len(V_ROWS) + len(O_PAIRS)) + 9
FEATURE_BLOCKS = ((0, 128), (128, 128), (256, 128), (384, 64))
SIDE_STEPS = ((1, 3, 5, 7, 9, 11), (1, 3, 5, 7), (1,), (1, 3, 5, 7))
LONG_CHUNKS = 2


def _dot(a, b):
    return lax.dot_general(a, b, (((1,), (0,)), ((), ())), preferred_element_type=F32)


def _dot_nt(a, b):
    return lax.dot_general(a, b, (((1,), (1,)), ((), ())), preferred_element_type=F32)


def _round_bf16(x):
    return x.astype(BF16).astype(F32)


def _pack(x):
    return pltpu.bitcast(x.astype(BF16), U32)


def _unpack(x):
    return pltpu.bitcast(x, BF16)


def _dup_rows(w):
    return jnp.concatenate([w, w[DM:D]], axis=0)


def _sigmoid(x):
    return 1.0 / (1.0 + jnp.exp(-x))


def _fold8(x):
    return functools.reduce(jnp.add, [x[r:r + 8] for r in range(0, x.shape[0], 8)])


def _mean(acc):
    return jnp.sum(acc, axis=0, keepdims=True) * (1.0 / D)


def _inv_std(acc):
    return 1.0 / jnp.sqrt(_mean(acc) + EPS)


def _group8(x, op, lane):
    for s in (1, 2, 4):
        partner = jnp.where((lane & s) == 0, pltpu.roll(x, 128 - s, 1), pltpu.roll(x, s, 1))
        x = op(x, partner)
    return x


def _start_of(index, size):
    return index * size if isinstance(index, int) else pl.multiple_of(index * size, size)


def _run(task):
    for _ in task:
        pass


def _wait(copies):
    for copy in copies:
        copy.wait()


def _kernel(xT_hbm, mem0_hbm, wq_hbm, wk_hbm, wv_hbm, woT_hbm, wr_hbm, wg_hbm, wu_hbm,
            wdT_hbm, c_hbm, wmod_hbm, out_hbm,
            xT, mem0, wqs, wks, wvs, wos, stage, wq_heads, part, part_tail, wr, wg, wu, wdT, c, wmod,
            ab, qtail, vtail, cols, hs, ao, cur, late, late_q, outv, h2s, sems, out_sems):
    started = []

    def start(src, dst):
        copy = pltpu.make_async_copy(src, dst, sems.at[len(started)])
        started.append(copy)
        copy.start()
        return [copy]

    def start_half(src, r0, n, e, dst):
        return start(src.at[pl.ds(r0, n), pl.ds(e * 128, 128)], dst.at[pl.ds(0, n)])

    def start_tokens(t0, n):
        return start(xT_hbm.at[:, pl.ds(t0, n)], xT.at[:, pl.ds(t0, n)])

    def start_values(ci):
        r0, n = V_ROWS[ci]
        return sum((start_half(wv_hbm, r0 * H, n * H, e, wvs[ci][e]) for e in range(2)), [])

    cp_q, cp_k = [], []
    for e in range(2):
        cp_q.append(start_half(wq_hbm, 0, D * H, e, wqs[e]))
        cp_k.append([start_half(wk_hbm, r0 * H, n * H, e, buf)
                     for (r0, n), buf in zip(K_ROWS, wks[e])])
    cp_v = [start_values(0)]
    cp_o = [sum((start_half(woT_hbm, 2 * p0 * D, 2 * n * D, e, buf[e]) for e in range(2)), [])
            for (p0, n), buf in zip(O_PAIRS, wos)]
    cp_v.append(start_values(1))
    cp_small = (start(c_hbm, c) + start(mem0_hbm, mem0) + start(wr_hbm, wr)
                + start(wmod_hbm, wmod) + start_tokens(0, 2 * G))
    cp_tokens = start_tokens(2 * G, S - 2 * G)
    cp_ffn = start(wg_hbm, wg) + start(wu_hbm, wu) + start(wdT_hbm, wdT)

    def as_words(dst, src):
        dst[:src.shape[0] // 2] = pltpu.bitcast(src[...], U32)
        return dst

    def head_pair(words, p, n):
        w32 = words[pl.ds(p, n, stride=H // 2), :]
        even = pltpu.bitcast(w32 << 16, F32).astype(BF16)
        odd = pltpu.bitcast(w32 & np.uint32(0xFFFF0000), F32).astype(BF16)
        return even, odd

    def fold(lhs, rhs):
        pad = -lhs[0].shape[0] % 128
        main = [_dot_nt(l, r[:DM]) for l, r in zip(lhs, rhs)]
        tail = [_dot_nt(r[DM:], jnp.concatenate([l, l[:pad]], axis=0) if pad else l)
                for l, r in zip(lhs, rhs)]
        return main + [jnp.concatenate(tail, axis=0)]

    def store_folded(kv, p, r0, even, odd, tail):
        n = even.shape[0]
        m = min(n, DM - r0)
        tail = tail.T[:n]
        rows = slice(r0 // 2, (r0 + m) // 2)
        for j in range(3):
            c0 = kv * HALF + j * H + 2 * p
            ab[c0, rows] = _pack(even[:m, j * 128:(j + 1) * 128])
            ab[c0 + 1, rows] = _pack(odd[:m, j * 128:(j + 1) * 128])
        ab[kv * HALF + 3 * H + p, rows] = _pack(tail[:m])
        if m == n:
            return
        if kv == 0:
            corner = jnp.concatenate([tail[m:], pltpu.roll(tail[m:], 64, 1)], axis=0)
            both = jnp.concatenate([jnp.concatenate([even[m:], odd[m:]], axis=0), corner], axis=1)
            qtail[p] = _pack(both.T[:D])
            return
        for j in range(3):
            vtail[j, 64 * p:64 * p + 64] = _pack(jnp.concatenate(
                [even[m:, j * 128:(j + 1) * 128], odd[m:, j * 128:(j + 1) * 128]], axis=0))
        left = lax.broadcasted_iota(jnp.int32, (D - DM, 128), 1) < 64
        vtail[3, 64 * p:64 * p + 64] = _pack(jnp.concatenate(
            [jnp.where(left, tail[m:], 0.0), jnp.where(left, 0.0, tail[m:])], axis=0))

    for e in range(2):
        _wait(cp_q[e])
        for ci, (r0, n) in enumerate(K_ROWS):
            if ci == 0:
                q_words = as_words(stage[0], wqs[e])
            _wait(cp_k[e][ci])
            k_words = as_words(stage[1], wks[e][ci])
            for p in range(H // 2):
                if ci == 0:
                    rhs = head_pair(q_words, p, D)
                    for odd in range(2):
                        wq_heads[2 * p + odd] = pltpu.bitcast(rhs[odd], U32)
                else:
                    rhs = [_unpack(wq_heads[2 * p + odd]) for odd in range(2)]
                ms = fold(head_pair(k_words, p, n), rhs)
                slots = [part.at[2 * p, r0:r0 + n], part.at[2 * p + 1, r0:r0 + n],
                         part_tail.at[ci, p, :, :ms[2].shape[1]]]
                if e == 0:
                    for slot, x in zip(slots, ms):
                        slot[...] = x
                else:
                    store_folded(0, p, r0, *(
                        (slot[...] + x) * E ** -0.5 for slot, x in zip(slots, ms)))

    for ci, (r0, n) in enumerate(V_ROWS):
        _wait(cp_v[ci])
        v_words = [as_words(stage[e], wvs[ci][e]) for e in range(2)]
        for (p0, count), buf, copies in zip(O_PAIRS, wos, cp_o):
            if ci == 0:
                _wait(copies)
            for p in range(count):
                lhs = [head_pair(v_words[e], p0 + p, n) for e in range(2)]
                lhs = [jnp.concatenate([lhs[e][odd] for e in range(2)], axis=1)
                       for odd in range(2)]
                rhs = [jnp.concatenate([buf[e][h * D:(h + 1) * D, :] for e in range(2)], axis=1)
                       for h in (2 * p, 2 * p + 1)]
                store_folded(1, p0 + p, r0, *fold(lhs, rhs))

    _wait(cp_small)
    cond = c[...].astype(F32)
    mod = _round_bf16(_dot(jnp.broadcast_to(cond * _sigmoid(cond), (8, D)), wmod[...]))
    mod = jnp.broadcast_to(mod[0:1], (128, 6 * D)).T
    for n in range(6):
        col = mod[n * D:(n + 1) * D]
        cols[n] = _round_bf16(1.0 + col) if n % 3 == 1 else col
    router = jnp.concatenate(
        [wr[...].astype(F32).reshape(1, D), jnp.zeros((1, DP - D), F32)], axis=1)
    cols[6] = jnp.broadcast_to(router, (128, DP)).T[:D]

    SUM, SQ, SCORE, SQ2 = (pl.ds(D + 8 * n, 8) for n in range(4))

    def modulate(g):
        t = pl.ds(_start_of(g, G), G)
        hs[4, SUM, :] = sum(_fold8(xT[r:r + n, t].astype(F32)) for r, n in FEATURE_BLOCKS)
        yield
        m = _mean(hs[4, SUM, :])
        ds = [xT[r:r + n, t].astype(F32) - m for r, n in FEATURE_BLOCKS]
        hs[4, SQ, :] = sum(_fold8(d * d) for d in ds)
        yield
        inv = _inv_std(hs[4, SQ, :])
        for j, (r, n) in enumerate(FEATURE_BLOCKS):
            h = (xT[r:r + n, t].astype(F32) - m) * inv * cols[1, r:r + n] + cols[0, r:r + n]
            if n < 128:
                h = jnp.concatenate([h, h], axis=0)
            hs[j, t, :] = h.T
            yield

    def finish(g, scores):
        t = pl.ds(_start_of(g, G), G)
        acc = jnp.zeros((8, 128), F32)
        for j, (r, n) in enumerate(FEATURE_BLOCKS):
            a = ao[t, 128 * j:128 * j + 128].T[:n]
            x1 = xT[r:r + n, t].astype(F32) + cols[2, r:r + n] * a
            hs[4, r:r + n, :] = x1
            acc = acc + _fold8(x1)
            yield
        m = _mean(acc)
        ds = [hs[4, r:r + n, :] - m for r, n in FEATURE_BLOCKS]
        hs[4, SQ2, :] = sum(_fold8(d * d) for d in ds)
        yield
        inv = _inv_std(hs[4, SQ2, :])
        acc = jnp.zeros((8, 128), F32)
        for r, n in FEATURE_BLOCKS:
            x1 = hs[4, r:r + n, :]
            h2 = (x1 - m) * inv * cols[4, r:r + n] + cols[3, r:r + n]
            hs[4, SCORE, :] = acc + _fold8(h2 * cols[6, r:r + n])
            outv[r:r + n, t] = (x1 + cols[5, r:r + n] * (h2 + h2 * 0.0)).astype(BF16)
            h2s[g, r // 2:(r + n) // 2] = _pack(h2)
            yield
            acc = hs[4, SCORE, :]
        scores.append(_round_bf16(jnp.sum(acc, axis=0, keepdims=True)))

    lane1 = lax.broadcasted_iota(jnp.int32, (1, 128), 1)

    def better(r, g, best, best_idx):
        take = (r > best) & (g >= 0)
        return jnp.where(take, r, best), jnp.where(take, lane1 + g * G, best_idx)

    lane8 = lax.broadcasted_iota(jnp.int32, (8, 128), 1)
    lane40 = lax.broadcasted_iota(jnp.int32, (M + SEG, 128), 1)
    row40 = lax.broadcasted_iota(jnp.int32, (M + SEG, 128), 0)

    def weights(ref, tiles):
        return jnp.concatenate([_unpack(ref[t]) for t in tiles], axis=1)

    def heads4(o, i):
        return _pack(jnp.concatenate(
            [o[8 * i:8 * i + 8, 128 * q:128 * q + 128] for q in range(4)], axis=0))

    def pairs(o, i, qs):
        parts = []
        for q in qs:
            x = o[8 * i:8 * i + 8, 128 * q:128 * q + 128]
            parts.append(jnp.where(lane8 < 64, x, 0.0))
            parts.append(jnp.where(lane8 < 64, 0.0, x))
        return _pack(jnp.concatenate(parts, axis=0))

    def keep(o, kv, chunk):
        j, cq = divmod(chunk, 4)
        n = 16 if j < 3 else 32
        for t in range(4):
            cur[kv, j, 64 * t + n * cq:64 * t + n * (cq + 1), :] = (
                heads4(o, t) if j < 3 else pairs(o, t, range(4)))

    def keep_late(o, par, kv, j, cq):
        for i in range(4):
            late[par, i, kv, j, 16 * cq:16 * cq + 16, :] = heads4(o, i)

    def project(lhs, kv, chunk):
        keep(_dot(lhs[:, :DM], weights(ab, [kv * HALF + 4 * chunk + q for q in range(4)])),
             kv, chunk)

    def project_late(lhs, par, cq, chunk):
        if chunk < 6:
            kv, j = divmod(chunk, 3)
            o = _dot(lhs[:, :DM], weights(ab, [kv * HALF + j * H + 4 * cq + q for q in range(4)]))
            keep_late(o, par, kv, j, cq)
        else:
            o = _dot(lhs[:, :DM], weights(ab, [kv * HALF + 3 * H + 2 * cq + q
                                               for kv in range(2) for q in range(2)]))
            for i in range(4):
                for kv in range(2):
                    late[par, i, kv, 3, 16 * cq:16 * cq + 16, :] = pairs(
                        o, i, (2 * kv, 2 * kv + 1))

    def project_both(lhs, par, kv, j, cq):
        o = None
        for k in range(3):
            w = jnp.concatenate(
                [_unpack(ab[kv * HALF + j * H + 4 * cq + q, 64 * k:64 * k + 64]) for q in range(4)],
                axis=1)
            x = _dot(lhs[:, 128 * k:128 * k + 128], w)
            o = x if o is None else o + x
            if k == 2:
                keep(o[:32], kv, 4 * j + cq)
                keep_late(o[32:], par, kv, j, cq)
            yield

    def project_queries(lhs, half):
        return _dot(lhs, weights(qtail, range(4 * half, 4 * half + 4)))

    def token_rows(t0, n):
        return jnp.concatenate([hs[j, pl.ds(t0, n), :] for j in range(4)], axis=1)

    def late_rows(g):
        t0 = _start_of(g, G)
        rows = [token_rows(t0 + SEG * i + 24, 8) for i in range(4)]
        return jnp.concatenate(rows, axis=0).astype(BF16)[:, :D]

    def segment(g, i, mem, ahead, side):
        par = g & 1
        t0 = _start_of(4 * g + i, SEG)
        rows = jnp.concatenate([mem, token_rows(t0, SEG)], axis=0)
        lhs = rows[:32].astype(BF16)[:, :D]
        slot = lane40 >> 4
        tails = [pairs(rows, t, (3,)) for t in range(5)] + [jnp.zeros((8, 128), U32)] * 3
        zs = [_unpack(jnp.concatenate([tails[(u - p) % 8] for u in range(8)], axis=0))
              for p in range(8)]
        both = jnp.concatenate([lhs, ahead], axis=0)
        for chunk in range(14):
            if chunk == 6:
                q = jnp.concatenate([project_queries(lhs, half) for half in range(2)], axis=1)
                q = jnp.concatenate([q, late_q[par, 8 * i:8 * i + 8, :]], axis=0)
            project(lhs, 0, chunk)
            if chunk in SIDE_STEPS[i]:
                next(side, None)

        def long_passes():
            for j in range(LONG_CHUNKS):
                yield from project_both(both, 1 - par, 1, j, i)

        cover = long_passes()
        next(cover, None)
        raw = []
        for p in range(8):
            raw.append(_dot_nt(q[:, 128 * p:128 * p + 128], zs[p]))
            if p % 4 == 3:
                next(cover, None)
        s = None
        for j in range(4):
            x = _dot_nt(rows[:, 128 * j:128 * j + 128], _unpack(cur[0, j]))
            s = x if s is None else s + x
            next(cover, None)
        s = jnp.concatenate([s, _dot_nt(rows, weights(late.at[par, i, 0], range(4)))], axis=1)
        _run(cover)
        rest = [n for n in range(14) if n not in [4 * j + i for j in range(LONG_CHUNKS)]]
        for chunk in rest[:-1]:
            project(lhs, 1, chunk)

        ss = []
        for t in range(5):
            x = raw[0]
            for p in range(1, 8):
                x = jnp.where(slot == (p + t) % 8, raw[p], x)
            if t > 0:
                x = pltpu.roll(x, 128 - 16 * t, 1)
            st = s[:, t * 128:(t + 1) * 128] + x
            if t > 0:
                allowed = (row40 < M) | (row40 >= 8 * t + (lane40 & 7))
                st = jnp.where(allowed, st, MASKED)
            ss.append(st)
        mx = _group8(functools.reduce(jnp.maximum, ss), jnp.maximum, lane40)
        es = [jnp.exp(st - mx) for st in ss]
        inv = 1.0 / _group8(functools.reduce(jnp.add, es), jnp.add, lane40)
        ps = [e * inv for e in es]

        ys = [ps[0]] + [pltpu.roll(ps[t], 16 * t, 1) for t in range(1, 5)]
        z = []
        for p in range(8):
            x = ys[0]
            for t in range(1, 5):
                x = jnp.where(slot == (p + t) % 8, ys[t], x)
            z.append(_dot(x, zs[p]))
        project(lhs, 1, rest[-1])
        values = jnp.concatenate(
            [_unpack(jnp.concatenate([cur[1, j], late[par, i, 1, j]], axis=0)) for j in range(4)],
            axis=1)
        filler = [chunk for chunk in range(7) if not 3 <= chunk < 3 + LONG_CHUNKS]
        o = _dot(jnp.concatenate(z, axis=1), weights(vtail, range(4)))
        project_late(ahead, 1 - par, i, filler[0])
        o = o + _dot(jnp.concatenate(ps, axis=1), values)
        for chunk in filler[1:]:
            project_late(ahead, 1 - par, i, chunk)
        if i % 2 == 0:
            late_q[1 - par, :, 256 * i:256 * i + 512] = project_queries(ahead, i // 2)
        tail = o[:, DM:]
        o = jnp.concatenate([o[:, :DM], tail + pltpu.roll(tail, 64, 1)], axis=1)
        ao[pl.ds(t0, SEG), :] = o[M:]
        return o[:M]

    _run(modulate(0))
    _run(modulate(1))
    first = late_rows(0)
    for half in range(2):
        late_q[0, :, 512 * half:512 * half + 512] = project_queries(first, half)
    for cq in range(4):
        for chunk in range(7):
            project_late(first, 0, cq, chunk)
    ao[0:G, :] = jnp.zeros((G, DP), F32)
    _wait(cp_tokens)

    def out_copy(g, count, sem):
        t = pl.ds(_start_of(g, G), count * G)
        return pltpu.make_async_copy(outv.at[:, t], out_hbm.at[:, t], out_sems.at[sem])

    cp_out = [out_copy(0, NG - 2, 0), out_copy(NG - 2, 2, 1)]

    def group(g, carry):
        mem, best, best_idx = carry

        @pl.when(g == NG - 1)
        def _():
            cp_out[0].start()

        ahead = late_rows(jnp.minimum(g + 1, NG - 1))
        scores = []

        def side_work():
            yield from modulate(jnp.minimum(g + 2, NG - 1))
            yield from finish(jnp.maximum(g - 1, 0), scores)

        side = side_work()
        for i in range(4):
            mem = segment(g, i, mem, ahead, side)
        _run(side)
        return (mem,) + better(scores[0], g - 1, best, best_idx)

    mem = mem0[...].astype(F32)
    mem = jnp.concatenate([mem, mem[:, DM:D]], axis=1)
    _, best, best_idx = lax.fori_loop(
        0, NG, group, (mem, jnp.full((1, 128), -jnp.inf, F32), jnp.zeros((1, 128), jnp.int32)))
    scores = []
    _run(finish(NG - 1, scores))
    best, best_idx = better(scores[0], NG - 1, best, best_idx)
    cp_out[1].start()

    r_sel = jnp.max(best, axis=1, keepdims=True)
    idx = jnp.clip(jnp.min(jnp.where(best == r_sel, best_idx, S - 1)), 0, S - 1)
    g_sel, col = idx // G, idx % G
    pick = (lax.broadcasted_iota(jnp.int32, (8, G), 1) == col).astype(F32)
    x_sel = _dot_nt(pick, _dup_rows(_unpack(h2s[g_sel])))[:, :D]
    _wait(cp_ffn)
    gate = _dot(x_sel, wg[...])
    up = _dot(x_sel, wu[...])
    y = _dot_nt(gate * _sigmoid(gate) * up, _dup_rows(wdT[...]))[0:1] * _sigmoid(r_sel)
    y = jnp.broadcast_to(y, (128, DP)).T[:D]
    update = jnp.where(lax.broadcasted_iota(jnp.int32, (D, 128), 1) == col, y, 0.0)
    _wait(cp_out)
    t = pl.ds(_start_of(g_sel, G), G)
    outv[:, t] = (outv[:, t].astype(F32) + cols[5] * update).astype(BF16)
    last = out_copy(g_sel, 1, 2)
    last.start()
    last.wait()


@jax.jit
def pallas_adaLN_cond__memory_aug_recurrent_mem_tr__moe_arch_mod__prompt_kernel(
    A_x: jax.Array,
    A_mem0: jax.Array,
    A_Wq: jax.Array,
    A_Wk: jax.Array,
    A_Wv: jax.Array,
    A_Wo: jax.Array,
    A_seg_len: jax.Array,
    B_x: jax.Array,
    B_w_r: jax.Array,
    B_w_gate: jax.Array,
    B_w_up: jax.Array,
    B_w_down: jax.Array,
    c: jax.Array,
    w_mod: jax.Array,
):
    del A_seg_len, B_x
    hbm = pl.BlockSpec(memory_space=pl.ANY)

    def feature_rows(n):
        return pltpu.VMEM((n * H, 128), BF16)

    outT = pl.pallas_call(
        _kernel,
        out_shape=jax.ShapeDtypeStruct((D, S), BF16),
        in_specs=[hbm] * 12,
        out_specs=hbm,
        scratch_shapes=[
            pltpu.VMEM((D, S), BF16),
            pltpu.VMEM((M, D), BF16),
            [feature_rows(D)] * 2,
            [[feature_rows(n) for _, n in K_ROWS]] * 2,
            [[feature_rows(n)] * 2 for _, n in V_ROWS],
            [[pltpu.VMEM((2 * n * D, 128), BF16)] * 2 for _, n in O_PAIRS],
            [pltpu.VMEM(((D + 1) * H // 2, 128), U32)] * 2,
            pltpu.VMEM((H, D // 2, 128), U32),
            pltpu.VMEM((H, D, DM), F32),
            pltpu.VMEM((len(K_ROWS), H // 2, 128, DM), F32),
            pltpu.VMEM((D,), BF16),
            pltpu.VMEM((D, F), BF16),
            pltpu.VMEM((D, F), BF16),
            pltpu.VMEM((D, F), BF16),
            pltpu.VMEM((1, D), BF16),
            pltpu.VMEM((D, 6 * D), BF16),
            pltpu.VMEM((2 * HALF, DM // 2, 128), U32),
            pltpu.VMEM((H // 2, D // 2, 128), U32),
            pltpu.VMEM((4, H * 32, 128), U32),
            pltpu.VMEM((7, D, 128), F32),
            pltpu.VMEM((5, S, 128), F32),
            pltpu.VMEM((S, DP), F32),
            pltpu.VMEM((2, 4, 256, 128), U32),
            pltpu.VMEM((2, 4, 2, 4, 64, 128), U32),
            pltpu.VMEM((2, 32, 1024), F32),
            pltpu.VMEM((D, S), BF16),
            pltpu.VMEM((NG, D // 2, G), U32),
            pltpu.SemaphoreType.DMA((N_COPIES,)),
            pltpu.SemaphoreType.DMA((3,)),
        ],
        compiler_params=pltpu.CompilerParams(vmem_limit_bytes=100 * 1024 * 1024),
        name="adaln_rmt_mod",
    )(A_x.reshape(S, D).T, A_mem0.reshape(M, D), A_Wq.reshape(D * H, E), A_Wk.reshape(D * H, E),
      A_Wv.reshape(D * H, E), A_Wo.transpose(0, 2, 1).reshape(H * D, E), B_w_r, B_w_gate,
      B_w_up, B_w_down.T, c, w_mod)
    return outT.T.reshape(1, S, D)
```
